```python
import os as _os
_os.environ.setdefault("JAX_PLATFORMS", "cpu")
import jax
import jax.numpy as jnp

def _softmax(x, axis=-1):
    return jax.nn.softmax(x, axis=axis)
def _gelu(x):
    return jax.nn.gelu(x, approximate=True)
def _silu(x):
    return jax.nn.silu(x)
def _sigmoid(x):
    return jax.nn.sigmoid(x)
def _layernorm(x, axis=-1, eps=1e-5):
    m = jnp.mean(x, axis=axis, keepdims=True)
    v = jnp.var(x, axis=axis, keepdims=True)
    return (x - m) / jnp.sqrt(v + eps)
def _scatter_add(tgt, idx, src, axis=0):
    return tgt.at[idx].add(src)
def _segment_sum(src, seg, n):
    return jax.ops.segment_sum(src, seg, n)
class _Rng:
    def __init__(self, key):
        self._k = key
    def _next(self):
        self._k, sub = jax.random.split(self._k)
        return sub
    def normal(self, shape):
        return jax.random.normal(self._next(), shape, dtype=jnp.bfloat16)
    def randint(self, lo, hi, shape):
        return jax.random.randint(self._next(), shape, lo, hi, dtype=jnp.int32)
    def uniform(self, shape, lo=0.0, hi=1.0):
        return jax.random.uniform(self._next(), shape, jnp.bfloat16, lo, hi)
    def permutation(self, n):
        return jax.random.permutation(self._next(), n)


kernel_name = 'concat_heads__mha_block_cached__gqa_block_cached__near_ridge'

def setup_inputs():
    _rng = _Rng(jax.random.key(int.from_bytes(__import__("os").urandom(4), "little")))
    _w = (lambda a: (lambda t: t.astype(jnp.bfloat16) if jnp.issubdtype(t.dtype, jnp.floating) else t)(jnp.asarray(a)))
    def _A_setup():
        B, Sq, D = 8, 128, 512
        H, Sk, Dh = 32, 1024, 128
        return {
            "x": _w((lambda *s: _rng.normal(s) * 0.8)(B, Sq, D)),
            "k_cache": _w((lambda *s: _rng.normal(s) * 0.8)(B, H, Sk, Dh)),
            "v_cache": _w((lambda *s: _rng.normal(s) * 0.05)(B, H, Sk, Dh)),
            "wq": _w((lambda *s: _rng.normal(s) * 0.8)(D, H * Dh) * (D ** -0.5)),
            "wo": _w((lambda *s: _rng.normal(s) * 0.05)(H * Dh, D) * ((H * Dh) ** -0.5)),
        }
    _A_in = _A_setup()

    def _B_setup():
        B, Sq, D = 8, 128, 512
        Hq, Hkv, Sk, Dh = 32, 32, 1024, 128
        assert Hq % Hkv == 0, (Hq, Hkv)
        return {
            "x": _w((lambda *s: _rng.normal(s) * 0.8)(B, Sq, D)),
            "k_cache": _w((lambda *s: _rng.normal(s) * 0.8)(B, Hkv, Sk, Dh)),
            "v_cache": _w((lambda *s: _rng.normal(s) * 0.05)(B, Hkv, Sk, Dh)),
            "wq": _w((lambda *s: _rng.normal(s) * 0.8)(D, Hq * Dh) * (D ** -0.5)),
            "wo": _w((lambda *s: _rng.normal(s) * 0.05)(Hq * Dh, D) * ((Hq * Dh) ** -0.5)),
        }
    _B_in = _B_setup()

    return {
        "A_x": _A_in["x"],
        "A_k_cache": _A_in["k_cache"],
        "A_v_cache": _A_in["v_cache"],
        "A_wq": _A_in["wq"],
        "A_wo": _A_in["wo"],
        "B_x": _B_in["x"],
        "B_k_cache": _B_in["k_cache"],
        "B_v_cache": _B_in["v_cache"],
        "B_wq": _B_in["wq"],
        "B_wo": _B_in["wo"],
    }

def reference(A_x, A_k_cache, A_v_cache, A_wq, A_wo, B_x, B_k_cache, B_v_cache, B_wq, B_wo):
    def _A_ref(x, k_cache, v_cache, wq, wo):
        B, Sq, D = x.shape
        H, Dh = 32, 128
        q = (lambda x, *d: x.transpose(*d))((x @ wq).reshape(B, Sq, H, Dh), 0, 2, 1, 3)
        scores = jnp.einsum("bhqd,bhkd->bhqk", q, k_cache) * (Dh ** -0.5)
        p = _softmax(scores, axis=-1)
        o = jnp.einsum("bhqk,bhkd->bhqd", p, v_cache)
        return (lambda x, *d: x.transpose(*d))(o, 0, 2, 1, 3).reshape(B, Sq, H * Dh) @ wo

    def _B_ref(x, k_cache, v_cache, wq, wo):
        B, Sq, D = x.shape
        Hq, Dh = 32, 128
        Hkv = k_cache.shape[1]
        rep = Hq // Hkv
        q = (lambda x, *d: x.transpose(*d))((x @ wq).reshape(B, Sq, Hq, Dh), 0, 2, 1, 3)
        k = jnp.repeat(k_cache, rep, axis=1)
        v = jnp.repeat(v_cache, rep, axis=1)
        scores = jnp.einsum("bhqd,bhkd->bhqk", q, k) * (Dh ** -0.5)
        p = _softmax(scores, axis=-1)
        o = jnp.einsum("bhqk,bhkd->bhqd", p, v)
        return (lambda x, *d: x.transpose(*d))(o, 0, 2, 1, 3).reshape(B, Sq, Hq * Dh) @ wo

    a = _A_ref(A_x, A_k_cache, A_v_cache, A_wq, A_wo)
    b = _B_ref(B_x, B_k_cache, B_v_cache, B_wq, B_wo)
    return jnp.concatenate([a, b], axis=-1)
```

```python
import functools
import math

import jax
import jax.numpy as jnp
import jax.experimental.pallas as pl
import jax.experimental.pallas.tpu as pltpu

HG = 4
NB = 4


def _body(ax, ak, av, awq, awo, bx, bk, bv, bwq, bwo, out,
          xbuf, kbuf, vbuf, wqbuf, wobuf, qbuf, acc, obuf,
          xsem, ksem, vsem, wqsem, wosem, osem, *, B, S, D, H, DH):
    NG = H // HG
    NT = NG * B
    W = HG * DH
    c = (DH ** -0.5) * math.log2(math.e)
    f32, bf16 = jnp.float32, jnp.bfloat16

    def both(idx, n, fa, fb):
        pl.when(idx < n)(lambda: fa(idx))
        pl.when(idx >= n)(lambda: fb(idx - n))

    def kv_copy(src, buf, sem, t, slot):
        return pltpu.make_async_copy(
            src.at[t % B, pl.ds((t // B) * HG, HG)], buf.at[slot], sem.at[slot])

    def start_kv(t):
        slot = t % NB

        def go(k, v):
            def f(i):
                kv_copy(k, kbuf, ksem, i, slot).start()
                kv_copy(v, vbuf, vsem, i, slot).start()
            return f
        both(t, NT, go(ak, av), go(bk, bv))

    def wq_copy(src, g, slot):
        return pltpu.make_async_copy(
            src.at[:, pl.ds(pl.multiple_of(g * W, W), W)], wqbuf.at[slot], wqsem.at[slot])

    def wo_copy(src, g, slot):
        return pltpu.make_async_copy(
            src.at[pl.ds(pl.multiple_of(g * W, W), W)], wobuf.at[slot], wosem.at[slot])

    def start_w(G):
        slot = G % 2

        def go(wq, wo):
            def f(g):
                wq_copy(wq, g, slot).start()
                wo_copy(wo, g, slot).start()
            return f
        both(G, NG, go(awq, awo), go(bwq, bwo))

    def x_copy(p):
        return pltpu.make_async_copy((ax, bx)[p], xbuf.at[p], xsem.at[p])

    def o_copy(p, b):
        return pltpu.make_async_copy(
            obuf.at[p, pl.ds(pl.multiple_of(b * S, S), S)],
            out.at[pl.ds(pl.multiple_of(b * S, S), S), pl.ds(pl.multiple_of(p * D, D), D)],
            osem.at[p * B + b])

    x_copy(0).start()
    start_w(0)
    for i in range(NB - 1):
        start_kv(i)
    x_copy(1).start()
    x_copy(0).wait()

    def step(t, carry):
        G = t // B
        b = t % B
        p = G // NG
        g = G % NG
        slot = t % NB
        ws = G % 2

        @pl.when(t + NB - 1 < 2 * NT)
        def _():
            start_kv(t + NB - 1)

        @pl.when(b == 0)
        def _():
            pl.when(G + 1 < 2 * NG)(lambda: start_w(G + 1))
            pl.when(G == NG)(lambda: x_copy(1).wait())
            wq_copy(awq, 0, ws).wait()
            q = jnp.dot(xbuf[p], wqbuf[ws], preferred_element_type=f32)
            qbuf[...] = (q * c).astype(bf16)
            wo_copy(awo, 0, ws).wait()

        r = pl.ds(pl.multiple_of(b * S, S), S)
        kv_copy(ak, kbuf, ksem, 0, slot).wait()
        kv_copy(av, vbuf, vsem, 0, slot).wait()
        os = []
        for h in range(HG):
            s = jax.lax.dot_general(qbuf[r, h * DH:(h + 1) * DH], kbuf[slot, h],
                                    (((1,), (1,)), ((), ())), preferred_element_type=f32)
            m = jnp.max(s, -1, keepdims=True)
            e = jnp.exp2(s - m)
            l = jnp.sum(e, -1, keepdims=True)
            pv = jnp.dot(e.astype(bf16), vbuf[slot, h], preferred_element_type=f32)
            os.append((pv * (1.0 / l)).astype(bf16))
        y = jnp.dot(jnp.concatenate(os, axis=1), wobuf[ws], preferred_element_type=f32)

        @pl.when(g == 0)
        def _():
            acc[r, :] = y

        @pl.when((g > 0) & (g < NG - 1))
        def _():
            acc[r, :] += y

        @pl.when(g == NG - 1)
        def _():
            obuf[p, r, :] = (acc[r, :] + y).astype(bf16)
            o_copy(p, b).start()
        return carry

    jax.lax.fori_loop(0, 2 * NT, step, 0)
    for p in range(2):
        for b in range(B):
            o_copy(p, b).wait()


@jax.jit
def pallas_concat_heads__mha_block_cached__gqa_block_cached__near_ridge_kernel(
    A_x, A_k_cache, A_v_cache, A_wq, A_wo, B_x, B_k_cache, B_v_cache, B_wq, B_wo,
):
    B, S, D = A_x.shape
    _, H, SK, DH = A_k_cache.shape
    W = HG * DH
    bf16 = jnp.bfloat16
    dma = pltpu.SemaphoreType.DMA
    out = pl.pallas_call(
        functools.partial(_body, B=B, S=S, D=D, H=H, DH=DH),
        in_specs=[pl.BlockSpec(memory_space=pl.ANY)] * 10,
        out_specs=pl.BlockSpec(memory_space=pl.ANY),
        out_shape=jax.ShapeDtypeStruct((B * S, 2 * D), bf16),
        scratch_shapes=[
            pltpu.VMEM((2, B * S, D), bf16),
            pltpu.VMEM((NB, HG, SK, DH), bf16),
            pltpu.VMEM((NB, HG, SK, DH), bf16),
            pltpu.VMEM((2, D, W), bf16),
            pltpu.VMEM((2, W, D), bf16),
            pltpu.VMEM((B * S, W), bf16),
            pltpu.VMEM((B * S, D), jnp.float32),
            pltpu.VMEM((2, B * S, D), bf16),
            dma((2,)), dma((NB,)), dma((NB,)), dma((2,)), dma((2,)), dma((2 * B,)),
        ],
        compiler_params=pltpu.CompilerParams(vmem_limit_bytes=100 * 2 ** 20),
    )(A_x.reshape(B * S, D), A_k_cache, A_v_cache, A_wq, A_wo,
      B_x.reshape(B * S, D), B_k_cache, B_v_cache, B_wq, B_wo)
    return out.reshape(B, S, 2 * D)
```
